```python
import os as _os
_os.environ.setdefault("JAX_PLATFORMS", "cpu")
import jax
import jax.numpy as jnp

def _softmax(x, axis=-1):
    return jax.nn.softmax(x, axis=axis)
def _gelu(x):
    return jax.nn.gelu(x, approximate=True)
def _silu(x):
    return jax.nn.silu(x)
def _sigmoid(x):
    return jax.nn.sigmoid(x)
def _layernorm(x, axis=-1, eps=1e-5):
    m = jnp.mean(x, axis=axis, keepdims=True)
    v = jnp.var(x, axis=axis, keepdims=True)
    return (x - m) / jnp.sqrt(v + eps)
def _scatter_add(tgt, idx, src, axis=0):
    return tgt.at[idx].add(src)
def _segment_sum(src, seg, n):
    return jax.ops.segment_sum(src, seg, n)
class _Rng:
    def __init__(self, key):
        self._k = key
    def _next(self):
        self._k, sub = jax.random.split(self._k)
        return sub
    def normal(self, shape):
        return jax.random.normal(self._next(), shape, dtype=jnp.bfloat16)
    def randint(self, lo, hi, shape):
        return jax.random.randint(self._next(), shape, lo, hi, dtype=jnp.int32)
    def uniform(self, shape, lo=0.0, hi=1.0):
        return jax.random.uniform(self._next(), shape, jnp.bfloat16, lo, hi)
    def permutation(self, n):
        return jax.random.permutation(self._next(), n)


kernel_name = 'gated_mix__mha_block__softmax_full_mha__prompt'

def setup_inputs():
    _rng = _Rng(jax.random.key(int.from_bytes(__import__("os").urandom(4), "little")))
    _w = (lambda a: (lambda t: t.astype(jnp.bfloat16) if jnp.issubdtype(t.dtype, jnp.floating) else t)(jnp.asarray(a)))
    def _A_setup():
        B, S, D, H = 1, 2048, 448, 16
        return {
            "x": _w((lambda *s: _rng.normal(s) * 0.05)(B, S, D)),
            "wqkv": _w((lambda *s: _rng.normal(s) * 0.4)(D, 3 * D)),
            "wo": _w((lambda *s: _rng.normal(s) * 0.05)(D, D)),
        }
    _A_in = _A_setup()

    def _B_setup():
        B, S, D = 1, 2048, 448
        return {
            "x": _w((lambda *s: _rng.normal(s) * 0.05)(B, S, D)),
            "wqkv": _w((lambda *s: _rng.normal(s) * 0.4)(D, 3 * D)),
            "wo": _w((lambda *s: _rng.normal(s) * 0.05)(D, D)),
        }
    _B_in = _B_setup()

    return {
        "A_x": _A_in["x"],
        "A_wqkv": _A_in["wqkv"],
        "A_wo": _A_in["wo"],
        "B_x": _B_in["x"],
        "B_wqkv": _B_in["wqkv"],
        "B_wo": _B_in["wo"],
        "gate_w": _w((lambda *s: _rng.normal(s) * 0.05)(448) * 16.0),
    }

def reference(A_x, A_wqkv, A_wo, B_x, B_wqkv, B_wo, gate_w):
    def _A_ref(x, wqkv, wo):
        B, S, D = x.shape
        H = 16
        Dh = D // H
        qkv = (lambda x, *d: x.transpose(*d))((x @ wqkv).reshape(B, S, 3, H, Dh), 2, 0, 3, 1, 4)
        q, k, v = qkv[0], qkv[1], qkv[2]
        scores = jnp.einsum("bhqd,bhkd->bhqk", q, k) * (Dh ** -0.5)
        p = _softmax(scores, axis=-1)
        o = jnp.einsum("bhqk,bhkd->bhqd", p, v)
        return (lambda x, *d: x.transpose(*d))(o, 0, 2, 1, 3).reshape(B, S, D) @ wo

    def _B_ref(x, wqkv, wo):
        B, S, D = x.shape
        H = 16; Dh = D // H
        qkv = (lambda x, *d: x.transpose(*d))((x @ wqkv).reshape(B, S, 3, H, Dh), 2, 0, 3, 1, 4)
        q, k, v = qkv[0], qkv[1], qkv[2]
        scale = Dh ** -0.5
        scores = jnp.einsum("bhqd,bhkd->bhqk", q, k) * scale
        p = _softmax(scores, axis=-1)
        o = jnp.einsum("bhqk,bhkd->bhqd", p, v)
        return (lambda x, *d: x.transpose(*d))(o, 0, 2, 1, 3).reshape(B, S, D) @ wo

    x = A_x
    g = _sigmoid((x * gate_w).sum(-1, keepdims=True))
    a = _A_ref(x, A_wqkv, A_wo)
    b = _B_ref(x, B_wqkv, B_wo)
    return g * a + (1 - g) * b
```

```python
import math

import jax
import jax.numpy as jnp
import jax.experimental.pallas as pl
import jax.experimental.pallas.tpu as pltpu
from jax import lax

S, D, H, DH = 2048, 448, 16, 28
HP = 32
HB = H * HP
KL = 2 * H * HP - 128
GW = 4 * DH
W = 512
KC = 256
NJ = S // W
NC = S // KC
NP = 16
NT = 2 * H * NJ
NS = 8
W_CUTS = (0, 512, 2 * D, 3 * D)
F32, BF16 = jnp.float32, jnp.bfloat16


def _kernel(x_hbm, aw_hbm, awo_hbm, bw_hbm, bwo_hbm, gw_ref, out_hbm,
            x_buf, w_buf, wo_buf, wt_ref, wop_ref, tmp2_ref,
            k_ref, qm_ref, vt_ref, ot_ref, g_ref, oa_ref, stage_ref,
            s_ref, m_ref, in_sem, out_sem):
    def x_copy(c):
        p0 = pl.multiple_of(c * W, W)
        return pltpu.make_async_copy(x_hbm.at[0, :, pl.ds(p0, W)], x_buf.at[:, pl.ds(p0, W)], in_sem.at[c])

    wa_copy = [pltpu.make_async_copy(aw_hbm.at[:, W_CUTS[i]:W_CUTS[i + 1]], w_buf.at[0, :, W_CUTS[i]:W_CUTS[i + 1]],
                                     in_sem.at[NJ + i]) for i in range(3)]
    wb_copy = pltpu.make_async_copy(bw_hbm, w_buf.at[1], in_sem.at[NJ + 3])
    wo_copy = [pltpu.make_async_copy(w_h, wo_buf.at[b], in_sem.at[NJ + 4 + b]) for b, w_h in enumerate((awo_hbm, bwo_hbm))]
    later = ((x_copy(0),), (x_copy(1),), (x_copy(2), x_copy(3), wb_copy, wo_copy[0], wo_copy[1]))
    for cp in wa_copy:
        cp.start()

    qscale = (DH ** -0.5) * math.log2(math.e)

    def spread_heads(src_ref):
        parts = []
        for h in range(H):
            parts.append(src_ref[h * DH:(h + 1) * DH, :])
            parts.append(jnp.zeros((HP - DH, D), F32))
        return jnp.concatenate(parts, axis=0)

    def prep_w(b):
        for i in range(3):
            if b == 0:
                wa_copy[i].wait()
                for cp in later[i]:
                    cp.start()
            lo, hi = W_CUTS[i], W_CUTS[i + 1]
            wt_ref[lo:hi, :] = w_buf[b, :, lo:hi].astype(F32).T.astype(BF16)

    def prep_o(b):
        tmp2_ref[b] = wo_buf[b].astype(F32)
        wop_ref[:, b * HB:(b + 1) * HB] = spread_heads(tmp2_ref.at[b]).T.astype(BF16)

    def prep_gate():
        gcol = jnp.broadcast_to(gw_ref[...].astype(F32).reshape(1, D), (128, D)).T
        for n in range(S // 128):
            prod = x_buf[:, n * 128:(n + 1) * 128].astype(F32) * gcol
            part = jnp.sum(prod.reshape(D // 8, 8, 128), axis=0)
            logit = jnp.broadcast_to(jnp.sum(part, axis=0, keepdims=True), (8, 128))
            gate = jax.nn.sigmoid(logit)
            j, lo = divmod(n * 128, W)
            g_ref[j, :, lo:lo + 128] = gate
            g_ref[NJ + j, :, lo:lo + 128] = 1.0 - gate

    def project(c, b):
        @pl.when(b == 0)
        def _():
            x_copy(c).wait()

        p0 = pl.multiple_of(c * W, W)
        xt = x_buf[:, pl.ds(p0, W)]
        qkv = jnp.dot(wt_ref[...], xt, preferred_element_type=F32)
        qt = (qkv[0:D, :] * qscale).astype(BF16)
        r = lax.broadcasted_iota(jnp.int32, (GW, W), 0)
        for g in range(4):
            win = qt[g * GW:(g + 1) * GW, :]
            for j in range(4):
                t = (b * H + g * 4 + j) * NJ + c
                keep = jnp.logical_and(r >= j * DH, r < (j + 1) * DH)
                qm_ref[t, 0:GW, :] = jnp.where(keep, win, jnp.zeros_like(win))
                qm_ref[t, GW:128, :] = jnp.zeros((128 - GW, W), BF16)
            kk = qkv[D + g * GW:D + g * GW + 128, :].astype(BF16)
            k_ref[b * 4 + g, pl.ds(p0, W), :] = kk.T
        rr = lax.broadcasted_iota(jnp.int32, (HP, W), 0)
        fill = jnp.where(rr == DH, 1.0, 0.0)
        vall = jnp.concatenate([qkv[2 * D:3 * D, :], jnp.zeros((8, W), F32)], axis=0)
        for h in range(H):
            vh = jnp.where(rr < DH, vall[h * DH:h * DH + HP, :], fill).astype(BF16)
            for cc in range(W // KC):
                vt_ref[b * H + h, c * (W // KC) + cc] = vh[:, cc * KC:(cc + 1) * KC]

    def step(tn, tc, u, do_n=True, do_c=True, extra=None):
        mrun = acc = None
        if do_n:
            gn = lax.shift_right_logical(tn, 4)
            q = qm_ref[tn]
        if do_c:
            hc = lax.shift_right_logical(tc, 2)
            m = m_ref[u]
        for c in range(NC):
            if do_c:
                p = jnp.exp2(s_ref[u, c * KC:(c + 1) * KC, :].reshape(KC // 8, 8, W) - m[None])
                p = p.reshape(KC, W).astype(BF16)
                o = jnp.dot(vt_ref[hc, c], p, preferred_element_type=F32)
                acc = o if acc is None else acc + o
            if do_n:
                s = jnp.dot(k_ref[gn, c * KC:(c + 1) * KC, :], q, preferred_element_type=F32)
                s_ref[u, c * KC:(c + 1) * KC, :] = s
                mx = jnp.max(s.reshape(KC // 8, 8, W), axis=0)
                mrun = mx if mrun is None else jnp.maximum(mrun, mx)
            if extra is not None:
                extra(c)
        if do_n:
            m_ref[u] = jnp.broadcast_to(jnp.max(mrun, axis=0, keepdims=True), (8, W))
        if do_c:
            q0 = pl.multiple_of(lax.bitwise_and(tc, NJ - 1) * W, W)
            gate = g_ref[lax.shift_left(lax.shift_right_logical(tc, 6), 2) + lax.bitwise_and(tc, NJ - 1)]
            scale = gate / acc[DH:DH + 1, :]
            res = acc.reshape(HP // 8, 8, W) * scale[None]
            ot_ref[pl.ds(pl.multiple_of(hc * HP, HP), HP), pl.ds(q0, W)] = res.reshape(HP, W).astype(BF16)

    prep_w(0)

    def project_block(b, carry):
        lax.fori_loop(0, NJ, lambda c, cr: (project(c, b), cr)[1], 0)

        @pl.when(b == 0)
        def _():
            wb_copy.wait()
            step(0, 0, 0, do_c=False)
            step(1, 1, 1, do_c=False)
            prep_w(1)
        return carry

    lax.fori_loop(0, 2, project_block, 0)

    wo_copy[0].wait()
    wo_copy[1].wait()
    for u in range(2, NS):
        if u < 4:
            prep_o(u - 2)
        elif u == 4:
            prep_gate()
        step(u, u, u, do_c=False)

    def body(i, carry):
        t = NS * i
        for u in range(NS):
            step(t + u + NS, t + u, u)
        return carry

    lax.fori_loop(0, NT // NS - 1, body, 0)

    def out_copy(c, part):
        lo = part * 128
        return pltpu.make_async_copy(stage_ref.at[c, :, lo:lo + 128],
                                     out_hbm.at[0, :, c * W + lo:c * W + lo + 128], out_sem.at[4 * c + part])

    def out_piece(c, piece, late):
        n0 = c * W + (piece // 4) * 128
        r0 = (piece % 4) * GW
        k0, k1 = (KL, 2 * HB) if late else (0, KL)
        res = jnp.dot(wop_ref[r0:r0 + GW, k0:k1], ot_ref[k0:k1, n0:n0 + 128], preferred_element_type=F32)
        if not late:
            oa_ref[r0:r0 + GW, n0:n0 + 128] = res
        else:
            res = res + oa_ref[r0:r0 + GW, n0:n0 + 128]
            stage_ref[c, r0:r0 + GW, n0 - c * W:n0 - c * W + 128] = res.astype(BF16)
            if piece % 4 == 3:
                out_copy(c, piece // 4).start()

    assert NS == 2 * NJ
    for u in range(NS):
        def extra(kc, u=u):
            for slot in range(kc * NP // NC, (kc + 1) * NP // NC):
                if slot % 2 == 1:
                    e = u * (NP // 2) + slot // 2
                    out_piece(e // NP, e % NP, False)
                if u > NJ:
                    out_piece(u - NJ - 1, slot, True)
        step(0, NT - NS + u, u, do_n=False, extra=extra)
    for p in range(NP):
        out_piece(NJ - 1, p, True)
    for c in range(NJ):
        for part in range(4):
            out_copy(c, part).wait()


@jax.jit
def pallas_gated_mix__mha_block__softmax_full_mha__prompt_kernel(
    A_x: jax.Array,
    A_wqkv: jax.Array,
    A_wo: jax.Array,
    B_x: jax.Array,
    B_wqkv: jax.Array,
    B_wo: jax.Array,
    gate_w: jax.Array,
):
    assert A_x.shape == (1, S, D) and A_wqkv.shape == (D, 3 * D) and A_wo.shape == (D, D)
    any_spec = pl.BlockSpec(memory_space=pltpu.HBM)
    scratch = [
        pltpu.VMEM((D, S), BF16),
        pltpu.VMEM((2, D, 3 * D), BF16),
        pltpu.VMEM((2, D, D), BF16),
        pltpu.VMEM((3 * D, D), BF16),
        pltpu.VMEM((D, 2 * HB), BF16),
        pltpu.VMEM((2, D, D), F32),
        pltpu.VMEM((8, S, 128), BF16),
        pltpu.VMEM((NT, 128, W), BF16),
        pltpu.VMEM((2 * H, NC, HP, KC), BF16),
        pltpu.VMEM((2 * HB, S), BF16),
        pltpu.VMEM((2 * NJ, 8, W), F32),
        pltpu.VMEM((D, S), F32),
        pltpu.VMEM((NJ, D, W), BF16),
    ]
    scratch += [pltpu.VMEM((NS, S, W), F32), pltpu.VMEM((NS, 8, W), F32)]
    scratch += [pltpu.SemaphoreType.DMA((NJ + 6,)), pltpu.SemaphoreType.DMA((4 * NJ,))]
    out_t = pl.pallas_call(
        _kernel,
        in_specs=[any_spec] * 5 + [pl.BlockSpec(memory_space=pltpu.VMEM)],
        out_specs=any_spec,
        out_shape=jax.ShapeDtypeStruct((1, D, S), A_x.dtype),
        scratch_shapes=scratch,
        compiler_params=pltpu.CompilerParams(
            vmem_limit_bytes=100 * 2 ** 20,
            flags={"XLA_TPU_EVENLY_DISTRIBUTE_CRITICAL_NODES": True}),
    )(A_x.transpose(0, 2, 1), A_wqkv, A_wo, B_wqkv, B_wo, gate_w)
    return out_t.transpose(0, 2, 1)
```
